```python
import os as _os
_os.environ.setdefault("JAX_PLATFORMS", "cpu")
import jax
import jax.numpy as jnp

def _softmax(x, axis=-1):
    return jax.nn.softmax(x, axis=axis)
def _gelu(x):
    return jax.nn.gelu(x, approximate=True)
def _silu(x):
    return jax.nn.silu(x)
def _sigmoid(x):
    return jax.nn.sigmoid(x)
def _layernorm(x, axis=-1, eps=1e-5):
    m = jnp.mean(x, axis=axis, keepdims=True)
    v = jnp.var(x, axis=axis, keepdims=True)
    return (x - m) / jnp.sqrt(v + eps)
def _scatter_add(tgt, idx, src, axis=0):
    return tgt.at[idx].add(src)
def _segment_sum(src, seg, n):
    return jax.ops.segment_sum(src, seg, n)
class _Rng:
    def __init__(self, key):
        self._k = key
    def _next(self):
        self._k, sub = jax.random.split(self._k)
        return sub
    def normal(self, shape):
        return jax.random.normal(self._next(), shape, dtype=jnp.bfloat16)
    def randint(self, lo, hi, shape):
        return jax.random.randint(self._next(), shape, lo, hi, dtype=jnp.int32)
    def uniform(self, shape, lo=0.0, hi=1.0):
        return jax.random.uniform(self._next(), shape, jnp.bfloat16, lo, hi)
    def permutation(self, n):
        return jax.random.permutation(self._next(), n)


kernel_name = 'sequential_preLN__linear_attn_block__dense_activation_squared_relu__prompt'

def setup_inputs():
    _rng = _Rng(jax.random.key(int.from_bytes(__import__("os").urandom(4), "little")))
    _w = (lambda a: (lambda t: t.astype(jnp.bfloat16) if jnp.issubdtype(t.dtype, jnp.floating) else t)(jnp.asarray(a)))
    def _A_setup():
        B, S, D = 1, 2048, 576
        return {
            "x": _w((lambda *s: _rng.normal(s) * 0.05)(B, S, D)),
            "wqkv": _w((lambda *s: _rng.normal(s) * 0.1)(D, 3 * D)),
            "wo": _w((lambda *s: _rng.normal(s) * 0.05)(D, D)),
        }
    _A_in = _A_setup()

    def _B_setup():
        B, S, D, F = 1, 2048, 576, 4608
        return {
            "x": _w((lambda *s: _rng.normal(s) * 0.05)(B, S, D)),
            "w1": _w((lambda *s: _rng.normal(s) * 0.05)(D, F)),
            "b1": _w((lambda *s: _rng.normal(s) * 0.05)(F)),
            "w2": _w((lambda *s: _rng.normal(s) * 0.05)(F, D)),
            "b2": _w((lambda *s: _rng.normal(s) * 0.05)(D)),
        }
    _B_in = _B_setup()

    return {
        "A_x": _A_in["x"],
        "A_wqkv": _A_in["wqkv"],
        "A_wo": _A_in["wo"],
        "B_x": _B_in["x"],
        "B_w1": _B_in["w1"],
        "B_b1": _B_in["b1"],
        "B_w2": _B_in["w2"],
        "B_b2": _B_in["b2"],
    }

def reference(A_x, A_wqkv, A_wo, B_x, B_w1, B_b1, B_w2, B_b2):
    def _A_ref(x, wqkv, wo):
        B, S, D = x.shape
        H = 32; Dh = D // H
        qkv = (lambda x, *d: x.transpose(*d))((x @ wqkv).reshape(B, S, 3, H, Dh), 2, 0, 3, 1, 4)
        q, k, v = qkv[0], qkv[1], qkv[2]
        phi = lambda t: jnp.where(t > 0, t + 1, jnp.exp(t)) + 1e-6
        pq, pk = phi(q), phi(k)
        kv = jnp.einsum("bhsd,bhse->bhde", pk, v)
        z = jnp.einsum("bhsd->bhd", pk)
        num = jnp.einsum("bhqd,bhde->bhqe", pq, kv)
        den = jnp.einsum("bhqd,bhd->bhq", pq, z)[..., None] + 1e-6
        o = num / den
        return (lambda x, *d: x.transpose(*d))(o, 0, 2, 1, 3).reshape(B, S, D) @ wo

    def _B_ref(x, w1, b1, w2, b2):
        h = jnp.einsum("bsd,df->bsf", x, w1) + b1
        zero = jnp.zeros_like(h)
        r = jnp.where(h > zero, h, zero)
        h = r * r
        out = jnp.einsum("bsf,fd->bsd", h, w2) + b2
        return out

    x = A_x
    h = x + _A_ref(_layernorm(x, axis=-1), A_wqkv, A_wo)
    h2 = h + _B_ref(_layernorm(h, axis=-1), B_w1, B_b1, B_w2, B_b2)
    return h2
```

```python
import jax
import jax.numpy as jnp
from jax import lax
import jax.experimental.pallas as pl
import jax.experimental.pallas.tpu as pltpu

f32 = jnp.float32
bf16 = jnp.bfloat16
S, D, F, H, DH = 2048, 576, 4608, 32, 18
KP = 640
EPS_LN = 1e-5


def dot(a, b):
    return jnp.dot(a, b, preferred_element_type=f32)


def dot_nt(a, b):
    return lax.dot_general(a, b, (((1,), (1,)), ((), ())), preferred_element_type=f32)


def phi(t):
    return jnp.where(t > 0, t + 1.0, jnp.exp(t)) + 1e-6


def layernorm_T(xf):
    m = jnp.sum(xf, axis=0, keepdims=True) * (1.0 / D)
    xc = xf - m
    v = jnp.sum(xc * xc, axis=0, keepdims=True) * (1.0 / D)
    return xc * lax.rsqrt(v + EPS_LN)


ROWS = [(0, 144), (112, 272), (240, 400), (368, 528), (496, 576)]


def make(TN1=512, TN3=256, TN2=512, TF=512):
    NT1 = S // TN1
    NT3 = S // TN3
    NT2 = S // TN2
    NCH = F // TF

    def kernel(xT_hbm, wqkv_hbm, wo_hbm, w1_hbm, b1_hbm, w2T_hbm, b2_hbm, out_hbm,
               xT_v, wqkv_v, wo_v, w1_v, w2T_v, b1_v, b2_v,
               wqkT, w1T, ln1T, pqT, g_v, zmat, mT, hb, ln2T, ost, sems, osem):
        def cp(src, dst, i):
            return pltpu.make_async_copy(src, dst, sems.at[i])
        c_x = [cp(xT_hbm.at[:, pl.ds(i * TN1, TN1)], xT_v.at[:, pl.ds(i * TN1, TN1)], i) for i in range(NT1)]
        c_wk = cp(wqkv_hbm.at[:, pl.ds(512, 640)], wqkv_v.at[pl.ds(0, D), pl.ds(512, 640)], NT1)
        c_wq = cp(wqkv_hbm.at[:, pl.ds(0, 512)], wqkv_v.at[pl.ds(0, D), pl.ds(0, 512)], NT1 + 1)
        c_wv = cp(wqkv_hbm.at[:, pl.ds(1152, 576)], wqkv_v.at[pl.ds(0, D), pl.ds(1152, 576)], NT1 + 2)
        c_wo = cp(wo_hbm, wo_v, NT1 + 3)
        c_b1 = cp(b1_hbm, b1_v, NT1 + 4)
        c_b2 = cp(b2_hbm, b2_v, NT1 + 5)
        c_w1 = cp(w1_hbm, w1_v.at[pl.ds(0, D), :], NT1 + 6)
        c_w2 = cp(w2T_hbm, w2T_v, NT1 + 7)
        c_x[0].start()
        c_wk.start()
        for i in range(1, NT1):
            c_x[i].start()
        c_b1.start()
        c_b2.start()
        c_wq.start()
        c_wv.start()
        c_wo.start()
        c_w1.start()
        c_w2.start()

        r64 = lax.broadcasted_iota(jnp.int32, (KP - D, 128), 0)
        ones_blk = jnp.where(r64 == 0, 1.0, 0.0).astype(bf16)
        zero_blk = jnp.zeros((KP - D, 128), bf16)
        for j in range(S // 128):
            ln1T[D:KP, j * 128:(j + 1) * 128] = ones_blk
            ln2T[D:KP, j * 128:(j + 1) * 128] = ones_blk
        for j in range(14):
            w = 128 if j < 13 else 64
            wqkv_v[D:KP, j * 128:j * 128 + w] = zero_blk[:, :w]

        def ln1_tile(i):
            c_x[i].wait()
            for jj in range(TN1 // 128):
                c0 = i * TN1 + jj * 128
                xf = xT_v[:, c0:c0 + 128].astype(f32)
                ln1T[0:D, c0:c0 + 128] = layernorm_T(xf).astype(bf16)

        ln1_tile(0)
        c_wk.wait()
        for j in range(4, 9):
            wqkT[j * 128:(j + 1) * 128, :] = wqkv_v[:, j * 128:(j + 1) * 128].T
        for i in range(NT1):
            if i + 1 < NT1:
                ln1_tile(i + 1)
            c0 = i * TN1
            kT = dot(wqkT[D:2 * D, :], ln1T[:, c0:c0 + TN1])
            pk = phi(kT).astype(bf16)
            g = dot_nt(pk, ln1T[:, c0:c0 + TN1])
            if i == 0:
                g_v[...] = g
            else:
                g_v[...] += g

        c_wq.wait()
        for j in range(0, 4):
            wqkT[j * 128:(j + 1) * 128, :] = wqkv_v[:, j * 128:(j + 1) * 128].T
        c_wv.wait()
        c_wo.wait()
        g = g_v[...]
        zmat[...] = jnp.broadcast_to(g[:, D:D + 1], (D, 128))
        gb = g.astype(bf16)
        mparts = []
        for j, (r0, r1) in enumerate(ROWS):
            w = 128 if j < 4 else 64
            kv = dot(gb[r0:r1, :], wqkv_v[:, 2 * D + j * 128:2 * D + j * 128 + w])
            rr = lax.broadcasted_iota(jnp.int32, (r1 - r0, w), 0) + r0
            cc = lax.broadcasted_iota(jnp.int32, (r1 - r0, w), 1) + j * 128
            hr = (rr * 3641) >> 16
            hc = (cc * 3641) >> 16
            kvm = jnp.where(hr == hc, kv, 0.0).astype(bf16)
            mparts.append(dot(kvm, wo_v[j * 128:j * 128 + w, :]))
        pieces = []
        prev_tail = None
        for j, (r0, r1) in enumerate(ROWS):
            p = mparts[j]
            n = r1 - r0
            head_n = 0 if j == 0 else ROWS[j - 1][1] - r0
            tail_n = 0 if j == 4 else r1 - ROWS[j + 1][0]
            if head_n:
                pieces.append(prev_tail + p[0:head_n])
            pieces.append(p[head_n:n - tail_n])
            prev_tail = p[n - tail_n:n] if tail_n else None
        m = jnp.concatenate(pieces, axis=0).astype(bf16)
        mT[...] = m.T

        for i in range(NT1):
            c0 = i * TN1
            qT = dot(wqkT[0:D, :], ln1T[:, c0:c0 + TN1])
            pqT[:, c0:c0 + TN1] = phi(qT).astype(bf16)

        c_b1.wait()
        c_b2.wait()
        c_w1.wait()
        b1row = b1_v[...].reshape(1, F).astype(f32)
        for j in range(F // 128):
            bj = jnp.broadcast_to(b1row[:, j * 128:(j + 1) * 128], (KP - D, 128))
            w1_v[D:KP, j * 128:(j + 1) * 128] = jnp.where(r64 == 0, bj, 0.0).astype(bf16)
        for j in range(F // 128):
            w1T[j * 128:(j + 1) * 128, :] = w1_v[:, j * 128:(j + 1) * 128].T
        b2row = b2_v[...].reshape(1, D).astype(f32)
        b2cols = []
        for j in range(5):
            w = 128 if j < 4 else 64
            blk = jnp.broadcast_to(b2row[:, j * 128:j * 128 + w], (128, w))
            b2cols.append(blk.T)
        b2mat = jnp.concatenate(b2cols, axis=0)

        sub = lax.broadcasted_iota(jnp.int32, (8, 128), 0)
        for i in range(NT3):
            pqn_cols = []
            for jj in range(TN3 // 128):
                c0 = i * TN3 + jj * 128
                pq = pqT[:, c0:c0 + 128].astype(f32)
                t = pq * zmat[...]
                tg = [t[8 * v:8 * v + 8] for v in range(72)]
                rden = []
                for h in range(H):
                    a = (DH * h) // 8
                    o = (DH * h) % 8
                    e = o + DH - 16
                    ta = tg[a] if o == 0 else jnp.where(sub >= o, tg[a], 0.0)
                    tc = tg[a + 2] if e == 8 else jnp.where(sub < e, tg[a + 2], 0.0)
                    s = ta + tg[a + 1] + tc
                    den = jnp.sum(s, axis=0, keepdims=True) + 1e-6
                    rden.append(jnp.broadcast_to(1.0 / den, (8, 128)))
                outs = []
                for v in range(72):
                    hl = (8 * v) // DH
                    hh = (8 * v + 7) // DH
                    if hl == hh:
                        r = rden[hl]
                    else:
                        r = jnp.where(sub < (DH * hh - 8 * v), rden[hl], rden[hh])
                    outs.append(pq[8 * v:8 * v + 8] * r)
                pqn_cols.append(jnp.concatenate(outs, axis=0).astype(bf16))
            pqn = jnp.concatenate(pqn_cols, axis=1) if len(pqn_cols) > 1 else pqn_cols[0]
            c0 = i * TN3
            att = dot(mT[...], pqn)
            for jj in range(TN3 // 128):
                c1 = c0 + jj * 128
                hT = att[:, jj * 128:(jj + 1) * 128] + xT_v[:, c1:c1 + 128].astype(f32)
                ln2T[0:D, c1:c1 + 128] = layernorm_T(hT).astype(bf16)
                hb[:, c1:c1 + 128] = hT + b2mat

        c_w2.wait()

        def ffn_tile(i, carry):
            c0 = pl.multiple_of(i * TN2, TN2)
            slot = lax.rem(i, 2)
            acc = hb[:, pl.ds(c0, TN2)]
            l2 = ln2T[:, pl.ds(c0, TN2)]
            for j in range(NCH):
                h1 = dot(w1T[j * TF:(j + 1) * TF, :], l2)
                h1 = jnp.maximum(h1, 0.0)
                h1 = (h1 * h1).astype(bf16)
                acc = acc + dot(w2T_v[:, j * TF:(j + 1) * TF], h1)

            @pl.when(i >= 2)
            def _():
                pltpu.make_async_copy(ost.at[slot], out_hbm.at[:, pl.ds(c0, TN2)], osem.at[slot]).wait()
            ost[slot] = acc.astype(bf16)
            pltpu.make_async_copy(ost.at[slot], out_hbm.at[:, pl.ds(c0, TN2)], osem.at[slot]).start()
            return carry

        lax.fori_loop(0, NT2, ffn_tile, 0)
        for sl in range(2):
            pltpu.make_async_copy(ost.at[sl], out_hbm.at[:, pl.ds(0, TN2)], osem.at[sl]).wait()

    def fn(A_x, A_wqkv, A_wo, B_x, B_w1, B_b1, B_w2, B_b2):
        xT = jnp.swapaxes(A_x[0], 0, 1)
        w2T = jnp.swapaxes(B_w2, 0, 1)
        anyspec = pl.BlockSpec(memory_space=pl.ANY)
        out = pl.pallas_call(
            kernel,
            out_shape=jax.ShapeDtypeStruct((D, S), bf16),
            in_specs=[anyspec] * 7,
            out_specs=anyspec,
            scratch_shapes=[
                pltpu.VMEM((D, S), bf16),
                pltpu.VMEM((KP, 3 * D), bf16),
                pltpu.VMEM((D, D), bf16),
                pltpu.VMEM((KP, F), bf16),
                pltpu.VMEM((D, F), bf16),
                pltpu.VMEM((F,), bf16),
                pltpu.VMEM((D,), bf16),
                pltpu.VMEM((2 * D, KP), bf16),
                pltpu.VMEM((F, KP), bf16),
                pltpu.VMEM((KP, S), bf16),
                pltpu.VMEM((D, S), bf16),
                pltpu.VMEM((D, KP), f32),
                pltpu.VMEM((D, 128), f32),
                pltpu.VMEM((D, D), bf16),
                pltpu.VMEM((D, S), f32),
                pltpu.VMEM((KP, S), bf16),
                pltpu.VMEM((2, D, TN2), bf16),
                pltpu.SemaphoreType.DMA((NT1 + 8,)),
                pltpu.SemaphoreType.DMA((2,)),
            ],
            compiler_params=pltpu.CompilerParams(vmem_limit_bytes=100 * 1024 * 1024),
        )(xT, A_wqkv, A_wo, B_w1, B_b1, w2T, B_b2)
        return jnp.swapaxes(out, 0, 1)[None]

    return fn


_impl = make()


@jax.jit
def pallas_sequential_preLN__linear_attn_block__dense_activation_squared_relu__prompt_kernel(
    A_x: jax.Array,
    A_wqkv: jax.Array,
    A_wo: jax.Array,
    B_x: jax.Array,
    B_w1: jax.Array,
    B_b1: jax.Array,
    B_w2: jax.Array,
    B_b2: jax.Array,
):
    return _impl(A_x, A_wqkv, A_wo, B_x, B_w1, B_b1, B_w2, B_b2)
```

```python
import jax
import jax.numpy as jnp
from jax import lax
import jax.experimental.pallas as pl
import jax.experimental.pallas.tpu as pltpu

f32 = jnp.float32
bf16 = jnp.bfloat16
S, D, F, H, DH = 2048, 576, 4608, 32, 18
KP = 640
EPS_LN = 1e-5


def dot(a, b):
    return jnp.dot(a, b, preferred_element_type=f32)


def dot_nt(a, b):
    return lax.dot_general(a, b, (((1,), (1,)), ((), ())), preferred_element_type=f32)


def phi(t):
    return jnp.where(t > 0, t + 1.0, jnp.exp(t)) + 1e-6


def ln_stats(xf):
    m = jnp.sum(xf, axis=0, keepdims=True) * (1.0 / D)
    xc = xf - m
    v = jnp.sum(xc * xc, axis=0, keepdims=True) * (1.0 / D)
    return m, lax.rsqrt(v + EPS_LN)


def a_combos(A11, A12, A21, A22):
    return [A11 + A22, A21 + A22, A11, A22, A11 + A12, A21 - A11, A12 - A22]


def b_combos(B11, B12, B21, B22):
    return [B11 + B22, B11, B12 - B22, B21 - B11, B22, B11 + B12, B21 + B22]


def c_combos(M):
    M1, M2, M3, M4, M5, M6, M7 = M
    return (M1 + M4 - M5 + M7), (M3 + M5), (M2 + M4), (M1 - M2 + M3 + M6)


ROWS = [(0, 144), (112, 272), (240, 400), (368, 528), (496, 576)]


def make(R=384, WG=16):
    TA = 512
    NA = S // TA
    TN = 256
    TNh = TN // 2
    NT = S // TN
    N16 = S // 128
    TF = 2 * R
    NCH = F // TF
    RT = R // 128

    def kernel(xT_hbm, wqkv_hbm, wo_hbm, w1_hbm, b1_hbm, w2T_hbm, b2_hbm, out_hbm,
               xT_v, wqkv_v, wo_v, w1_v, w2T_v, b1_v, b2_v,
               wkT, wqP, pscr, ln1T, pkb, g_v, zmat, mT, pqb, pqnb, hb, b2m,
               l2c, l2r, w1a, w1r, w2c, mbuf, bbuf, accs, ost, stat, sems, osem):

        def cp(src, dst, i):
            return pltpu.make_async_copy(src, dst, sems.at[i])
        c_x = [None] + [cp(xT_hbm.at[:, pl.ds(i * TA, TA)], xT_v.at[i], i) for i in range(1, NA)]
        c_x0a = cp(xT_hbm.at[:, pl.ds(0, 256)], xT_v.at[0, :, pl.ds(0, 256)], 0)
        c_x0b = cp(xT_hbm.at[:, pl.ds(256, 256)], xT_v.at[0, :, pl.ds(256, 256)], NA + 8)
        c_wk = cp(wqkv_hbm.at[:, pl.ds(512, 256)], wqkv_v.at[pl.ds(0, D), pl.ds(512, 256)], NA)
        c_wk2 = cp(wqkv_hbm.at[:, pl.ds(768, 384)], wqkv_v.at[pl.ds(0, D), pl.ds(768, 384)], NA + 9)
        c_wq = cp(wqkv_hbm.at[:, pl.ds(0, 512)], wqkv_v.at[pl.ds(0, D), pl.ds(0, 512)], NA + 1)
        c_wv = cp(wqkv_hbm.at[:, pl.ds(1152, 576)], wqkv_v.at[pl.ds(0, D), pl.ds(1152, 576)], NA + 2)
        c_wo = cp(wo_hbm, wo_v, NA + 3)
        c_b1 = cp(b1_hbm, b1_v, NA + 4)
        c_b2 = cp(b2_hbm, b2_v, NA + 5)
        c_w1 = cp(w1_hbm, w1_v.at[pl.ds(0, D), :], NA + 6)
        c_w2 = cp(w2T_hbm, w2T_v, NA + 7)
        c_x0a.start()
        c_x0b.start()
        c_wk.start()
        c_wk2.start()
        for i in range(1, NA):
            c_x[i].start()
        for c in (c_w1, c_b1, c_b2, c_wq, c_wv, c_wo, c_w2):
            c.start()

        r64 = lax.broadcasted_iota(jnp.int32, (KP - D, 128), 0)
        ones_blk = jnp.where(r64 == 0, 1.0, 0.0).astype(bf16)
        zero_blk = jnp.zeros((KP - D, 128), bf16)
        for n in range(N16):
            ln1T[n, D:KP, :] = ones_blk
        for j in range(2):
            l2r[j, 64:128, :] = ones_blk
        for j in range(14):
            w = 128 if j < 13 else 64
            wqkv_v[D:KP, j * 128:j * 128 + w] = zero_blk[:, :w]
        for t in range(7):
            accs[t] = jnp.zeros((288, TNh), f32)

        def xcols(n):
            return xT_v[n // 4, :, (n % 4) * 128:(n % 4 + 1) * 128]

        def ln_stats_ref(load, slot):
            def vsum(x):
                return (x[0:16] + x[16:32]) + (x[32:48] + x[48:64])
            acc = None
            for g in range(0, D, 64):
                t = vsum(load(g, g + 64))
                acc = t if acc is None else acc + t
            m = jnp.sum(acc, axis=0, keepdims=True) * (1.0 / D)
            stat[slot, 0] = jnp.broadcast_to(m, (8, 128))
            acc = None
            for g in range(0, D, 64):
                xc = load(g, g + 64) - m
                t = vsum(xc * xc)
                acc = t if acc is None else acc + t
            r = lax.rsqrt(jnp.sum(acc, axis=0, keepdims=True) * (1.0 / D) + EPS_LN)
            stat[slot, 1] = jnp.broadcast_to(r, (8, 128))
            return m, r

        def LN1(i, jjs=(0, 1, 2, 3)):
            for jj in jjs:
                n = 4 * i + jj

                def ld(r0, r1):
                    return xT_v[n // 4, r0:r1, (n % 4) * 128:(n % 4 + 1) * 128].astype(f32)
                m, r = ln_stats_ref(ld, jj % 2)
                for g in range(0, D, 64):
                    ln1T[n, g:g + 64, :] = ((ld(g, g + 64) - m) * r).astype(bf16)

        def cat(xs, axis):
            return xs[0] if len(xs) == 1 else jnp.concatenate(xs, axis=axis)

        def KST(i, jjs=(0, 1, 2, 3), r0=0, r1=D):
            kT = dot(wkT[r0:r1, :], cat([ln1T[4 * i + jj] for jj in jjs], 1))
            pk = phi(kT).astype(bf16)
            for q, jj in enumerate(jjs):
                pkb[4 * i + jj, r0:r1, :] = pk[:, q * 128:(q + 1) * 128]

        def WKT(js):
            for j in js:
                tw = wqkv_v[:, j * 128:(j + 1) * 128].T
                if j == 4:
                    wkT[0:64, :] = tw[64:128]
                else:
                    wkT[(j - 4) * 128 - 64:(j - 3) * 128 - 64, :] = tw

        def GST(i):
            g = dot_nt(cat([pkb[4 * i + jj] for jj in range(4)], 1), cat([ln1T[4 * i + jj] for jj in range(4)], 1))
            if i == 0:
                g_v[...] = g
            else:
                g_v[...] += g

        def QST(t8, par):
            qT = dot(wqP[...], cat([ln1T[2 * t8 + jj] for jj in range(2)], 1))
            pq = phi(qT).astype(bf16)
            for jj in range(2):
                pqb[par, jj] = pq[:, jj * 128:(jj + 1) * 128]
            return qT

        def perm_rows(c):
            return cat([pscr[c, pl.ds(144 * blk + d, 8, stride=DH), :] for blk in range(4) for d in range(DH)], 0)

        def NST(par):
            for jj in range(2):
                for blk in range(4):
                    b0 = 144 * blk
                    pq = pqb[par, jj, b0:b0 + 144, :].astype(f32)
                    t = pq * zmat[b0:b0 + 144, :]
                    ts = [t[8 * d:8 * d + 8] for d in range(DH)]
                    while len(ts) > 1:
                        ts = [ts[k] + ts[k + 1] for k in range(0, len(ts) - 1, 2)] + ([ts[-1]] if len(ts) % 2 else [])
                    rden = 1.0 / (ts[0] + 1e-6)
                    pqnb[par, jj, b0:b0 + 144, :] = (pq * jnp.tile(rden, (DH, 1))).astype(bf16)

        def TST(t8, par, q4, half):
            att = dot(mT[...], cat([pqnb[par, jj] for jj in range(2)], 1))
            for jj in range(2):
                c0 = half * 256 + jj * 128
                hb[t8, jj] = att[:, jj * 128:(jj + 1) * 128] + xT_v[q4, :, c0:c0 + 128].astype(f32)
            return att

        def LST(t8):
            stats = [ln_stats_ref(lambda r0, r1, n=n: hb[t8, n, r0:r1, :], n) for n in range(2)]

            def nrm(r0, r1, n):
                m, r = stats[n]
                return (hb[t8, n, r0:r1, :] - m) * r
            for g in range(4):
                r0 = 64 * g
                bc = b_combos(nrm(r0, r0 + 64, 0), nrm(r0, r0 + 64, 1), nrm(256 + r0, 256 + r0 + 64, 0), nrm(256 + r0, 256 + r0 + 64, 1))
                for t in range(7):
                    l2c[t, r0:r0 + 64, :] = bc[t].astype(bf16)
            for n in range(2):
                l2r[n, 0:64, :] = nrm(512, 576, n).astype(bf16)

        def W1P(j, r):
            f1 = pl.multiple_of((2 * RT * j + r) * 128, 128)
            f2 = pl.multiple_of((2 * RT * j + RT + r) * 128, 128)
            for kk in range(2):
                A11 = w1_v[kk * 128:(kk + 1) * 128, pl.ds(f1, 128)].T.astype(f32)
                A12 = w1_v[(2 + kk) * 128:(3 + kk) * 128, pl.ds(f1, 128)].T.astype(f32)
                A21 = w1_v[kk * 128:(kk + 1) * 128, pl.ds(f2, 128)].T.astype(f32)
                A22 = w1_v[(2 + kk) * 128:(3 + kk) * 128, pl.ds(f2, 128)].T.astype(f32)
                for t, c in enumerate(a_combos(A11, A12, A21, A22)):
                    w1a[j, t, kk, r * 128:(r + 1) * 128, :] = c.astype(bf16)
            w1r[j, 0, r * 128:(r + 1) * 128, :] = w1_v[512:KP, pl.ds(f1, 128)].T
            w1r[j, 1, r * 128:(r + 1) * 128, :] = w1_v[512:KP, pl.ds(f2, 128)].T

        def W2P(j, r, toks, zdyn):
            f1 = pl.multiple_of((2 * RT * j + r) * 128, 128)
            f2 = pl.multiple_of((2 * RT * j + RT + r) * 128, 128)
            for g in range(288 // WG):
                r0 = WG * g
                A11 = w2T_v[r0:r0 + WG, pl.ds(f1, 128)].astype(f32)
                A12 = w2T_v[r0:r0 + WG, pl.ds(f2, 128)].astype(f32)
                A21 = w2T_v[288 + r0:288 + r0 + WG, pl.ds(f1, 128)].astype(f32)
                A22 = w2T_v[288 + r0:288 + r0 + WG, pl.ds(f2, 128)].astype(f32)
                msk = jnp.tile((pltpu.bitcast(toks[g], jnp.int32) & zdyn) != 0, (WG // 8, 1))
                A11 = jnp.where(msk, 0.0, A11)
                A22 = jnp.where(msk, 0.0, A22)
                for t, c in enumerate(a_combos(A11, A12, A21, A22)):
                    if t in (2, 3):
                        continue
                    w2c[j, t, r, r0:r0 + WG, :] = c.astype(bf16)

        c_x0a.wait()
        LN1(0, (0, 1))
        c_x0b.wait()
        LN1(0, (2, 3))
        c_wk.wait()
        WKT((4, 5))
        KST(0, (0, 1, 2, 3), 0, 192)
        c_wk2.wait()
        WKT((6, 7, 8))
        KST(0, (0, 1, 2, 3), 192, D)
        c_x[1].wait()
        GST(0)
        LN1(1)
        c_x[2].wait()
        c_x[3].wait()
        LN1(2)
        KST(1)
        LN1(3)
        GST(1)
        KST(2)
        GST(2)
        KST(3)

        for c in (c_w1, c_b1, c_b2, c_wq, c_wv, c_wo):
            c.wait()
        b1row = b1_v[...].reshape(1, F).astype(f32)
        for j in range(F // 128):
            bj = jnp.broadcast_to(b1row[:, j * 128:(j + 1) * 128], (KP - D, 128))
            w1_v[D:KP, j * 128:(j + 1) * 128] = jnp.where(r64 == 0, bj, 0.0).astype(bf16)
        for j in range(5):
            rows = 128 if j < 4 else 64
            tw = wqkv_v[:, j * 128:(j + 1) * 128].T.astype(f32)
            for c in range(5):
                pscr[c, j * 128:j * 128 + rows, :] = tw[0:rows, c * 128:(c + 1) * 128]
        for c in range(5):
            wqP[:, c * 128:(c + 1) * 128] = perm_rows(c).astype(bf16)
        GST(3)
        for p in range(NCH * RT):
            W1P(p // RT, p % RT)
        b2row = b2_v[...].reshape(1, D).astype(f32)
        for j in range(5):
            w = 128 if j < 4 else 64
            blk = jnp.broadcast_to(b2row[:, j * 128:j * 128 + w], (128, w))
            b2m[j * 128:j * 128 + w, :] = blk.T
        QST(0, 0)
        pscr[0] = jnp.broadcast_to(g_v[:, D:D + 1], (D, 128))
        zmat[...] = perm_rows(0)
        mparts = []
        for j, (r0, r1) in enumerate(ROWS):
            w = 128 if j < 4 else 64
            kv = dot(g_v[r0:r1, :].astype(bf16), wqkv_v[:, 2 * D + j * 128:2 * D + j * 128 + w])
            rr = lax.broadcasted_iota(jnp.int32, (r1 - r0, w), 0) + r0
            cc = lax.broadcasted_iota(jnp.int32, (r1 - r0, w), 1) + j * 128
            kvm = jnp.where(((rr * 3641) >> 16) == ((cc * 3641) >> 16), kv, 0.0).astype(bf16)
            mparts.append(kvm)
        QST(1, 1)
        pieces = []
        prev_tail = None
        for j, (r0, r1) in enumerate(ROWS):
            w = 128 if j < 4 else 64
            p = dot(mparts[j], wo_v[j * 128:j * 128 + w, :])
            n = r1 - r0
            head_n = 0 if j == 0 else ROWS[j - 1][1] - r0
            tail_n = 0 if j == 4 else r1 - ROWS[j + 1][0]
            if head_n:
                pieces.append(prev_tail + p[0:head_n])
            pieces.append(p[head_n:n - tail_n])
            prev_tail = p[n - tail_n:n] if tail_n else None
        m = jnp.concatenate(pieces, axis=0)
        for c in range(5):
            w = 128 if c < 4 else 64
            pscr[c, :, 0:w] = m[:, c * 128:c * 128 + w]
        for c in range(5):
            w = 128 if c < 4 else 64
            mT[c * 128:c * 128 + w, :] = perm_rows(c)[:, 0:w].astype(bf16).T
        NST(0)

        c_w2.wait()

        def bbody(u, carry):
            tk = []
            for half in range(2):
                a = TST(2 * u + half, half, u, half)
                NST(1 - half)
                q = QST(2 * u + 2 + half, half)
                for v in (a, q):
                    tk += [v[8 * ((k * 72) // 27):8 * ((k * 72) // 27) + 8, 128 * (k % 2):128 * (k % 2) + 128] for k in range(27)]
            ng = 288 // WG
            for p in range(6):
                W2P(2 * u + p // RT, p % RT, [tk[((p * ng + g) * 108) // (6 * ng)] for g in range(ng)], u >> 31)
            return carry
        lax.fori_loop(0, 3, bbody, 0)
        TST(6, 0, 3, 0)
        NST(1)
        LST(0)
        TST(7, 1, 3, 1)


        def out_copy(i, slot):
            return pltpu.make_async_copy(ost.at[slot], out_hbm.at[:, pl.ds(pl.multiple_of(i * TN, TN), TN)], osem.at[slot])

        def FC(i, slot):
            C11, C12, C21, C22 = c_combos([accs[t] for t in range(7)])
            ost[slot, 0:288, 0:TNh] = (C11 + hb[i, 0, 0:288, :] + b2m[0:288, :]).astype(bf16)
            ost[slot, 0:288, TNh:TN] = (C12 + hb[i, 1, 0:288, :] + b2m[0:288, :]).astype(bf16)
            ost[slot, 288:D, 0:TNh] = (C21 + hb[i, 0, 288:D, :] + b2m[288:D, :]).astype(bf16)
            ost[slot, 288:D, TNh:TN] = (C22 + hb[i, 1, 288:D, :] + b2m[288:D, :]).astype(bf16)

        def tile(i, carry):
            pslot = lax.rem(i + 1, 2)

            @pl.when(i >= 3)
            def _():
                out_copy(i - 3, pslot).wait()
            FC(jnp.maximum(i - 1, 0), pslot)

            def S1(j):
                sl = j % 2
                for t in range(7):
                    mbuf[sl, t] = dot(w1a[j, t, 0], l2c[t, 0:128, :]) + dot(w1a[j, t, 1], l2c[t, 128:256, :])
                mbuf[sl, 7] = dot(w1r[j, 0], l2r[0])
                mbuf[sl, 8] = dot(w1r[j, 0], l2r[1])
                mbuf[sl, 9] = dot(w1r[j, 1], l2r[0])
                mbuf[sl, 10] = dot(w1r[j, 1], l2r[1])

            def S2(j):
                sl = j % 2
                C = list(c_combos([mbuf[sl, t] for t in range(7)]))
                C = [C[q] + mbuf[sl, 7 + q] for q in range(4)]
                Hq = [jnp.maximum(c, 0.0) for c in C]
                Hq = [h * h for h in Hq]
                bc = b_combos(*Hq)
                for t in range(7):
                    bbuf[sl, t] = bc[t].astype(bf16)

            def S3(j):
                sl = j % 2
                for t in range(7):
                    def lhs(r):
                        if t == 2:
                            return w2T_v[0:288, (2 * RT * j + r) * 128:(2 * RT * j + r + 1) * 128]
                        if t == 3:
                            return w2T_v[288:D, (2 * RT * j + RT + r) * 128:(2 * RT * j + RT + r + 1) * 128]
                        return w2c[j, t, r]
                    mm = dot(lhs(0), bbuf[sl, t, 0:128, :])
                    for r in range(1, RT):
                        mm = mm + dot(lhs(r), bbuf[sl, t, r * 128:(r + 1) * 128, :])
                    if j == 0:
                        accs[t] = mm
                    else:
                        accs[t] += mm
            steps = []
            for step in range(NCH + 2):
                if step - 2 >= 0:
                    steps.append((S3, step - 2))
                if 0 <= step - 1 < NCH:
                    steps.append((S2, step - 1))
                if step < NCH:
                    steps.append((S1, step))
            for fn_, j in steps:
                fn_(j)
                if fn_ is S1 and j == NCH - 1:
                    LST(jnp.minimum(i + 1, NT - 1))

            @pl.when(i >= 1)
            def _():
                out_copy(i - 1, pslot).start()
            return carry

        lax.fori_loop(0, NT, tile, 0)
        out_copy(NT - 3, 1).wait()
        M = [accs[t] for t in range(7)]
        C11, C12, C21, C22 = c_combos(M)
        c0 = (NT - 1) * TN
        top = pltpu.make_async_copy(ost.at[1, pl.ds(0, 288)], out_hbm.at[pl.ds(0, 288), pl.ds(c0, TN)], osem.at[1])
        bot = pltpu.make_async_copy(ost.at[1, pl.ds(288, 288)], out_hbm.at[pl.ds(288, 288), pl.ds(c0, TN)], osem.at[2])
        ost[1, 0:288, 0:TNh] = (C11 + hb[NT - 1, 0, 0:288, :] + b2m[0:288, :]).astype(bf16)
        ost[1, 0:288, TNh:TN] = (C12 + hb[NT - 1, 1, 0:288, :] + b2m[0:288, :]).astype(bf16)
        top.start()
        ost[1, 288:D, 0:TNh] = (C21 + hb[NT - 1, 0, 288:D, :] + b2m[288:D, :]).astype(bf16)
        ost[1, 288:D, TNh:TN] = (C22 + hb[NT - 1, 1, 288:D, :] + b2m[288:D, :]).astype(bf16)
        bot.start()
        out_copy(NT - 2, 0).wait()
        top.wait()
        bot.wait()

    def fn(A_x, A_wqkv, A_wo, B_x, B_w1, B_b1, B_w2, B_b2):
        xT = jnp.swapaxes(A_x[0], 0, 1)
        w2T = jnp.swapaxes(B_w2, 0, 1)
        anyspec = pl.BlockSpec(memory_space=pl.ANY)
        out = pl.pallas_call(
            kernel,
            out_shape=jax.ShapeDtypeStruct((D, S), bf16),
            in_specs=[anyspec] * 7,
            out_specs=anyspec,
            scratch_shapes=[
                pltpu.VMEM((NA, D, TA), bf16),
                pltpu.VMEM((KP, 3 * D), bf16),
                pltpu.VMEM((D, D), bf16),
                pltpu.VMEM((KP, F), bf16),
                pltpu.VMEM((D, F), bf16),
                pltpu.VMEM((F,), bf16),
                pltpu.VMEM((D,), bf16),
                pltpu.VMEM((D, KP), bf16),
                pltpu.VMEM((D, KP), bf16),
                pltpu.VMEM((5, D, 128), f32),
                pltpu.VMEM((N16, KP, 128), bf16),
                pltpu.VMEM((N16, D, 128), bf16),
                pltpu.VMEM((D, KP), f32),
                pltpu.VMEM((D, 128), f32),
                pltpu.VMEM((D, D), bf16),
                pltpu.VMEM((2, 2, D, 128), bf16),
                pltpu.VMEM((2, 2, D, 128), bf16),
                pltpu.VMEM((NT, 2, D, 128), f32),
                pltpu.VMEM((D, 128), f32),
                pltpu.VMEM((7, 256, TNh), bf16),
                pltpu.VMEM((2, 128, 128), bf16),
                pltpu.VMEM((NCH, 7, 2, R, 128), bf16),
                pltpu.VMEM((NCH, 2, R, 128), bf16),
                pltpu.VMEM((NCH, 7, RT, 288, 128), bf16),
                pltpu.VMEM((2, 11, R, TNh), f32),
                pltpu.VMEM((2, 7, R, TNh), bf16),
                pltpu.VMEM((7, 288, TNh), f32),
                pltpu.VMEM((2, D, TN), bf16),
                pltpu.VMEM((2, 2, 8, 128), f32),
                pltpu.SemaphoreType.DMA((NA + 10,)),
                pltpu.SemaphoreType.DMA((3,)),
            ],
            compiler_params=pltpu.CompilerParams(vmem_limit_bytes=100 * 1024 * 1024),
        )(xT, A_wqkv, A_wo, B_w1, B_b1, w2T, B_b2)
        return jnp.swapaxes(out, 0, 1)[None]

    return fn


_impl = make()


@jax.jit
def pallas_sequential_preLN__linear_attn_block__dense_activation_squared_relu__prompt_kernel(
    A_x: jax.Array,
    A_wqkv: jax.Array,
    A_wo: jax.Array,
    B_x: jax.Array,
    B_w1: jax.Array,
    B_b1: jax.Array,
    B_w2: jax.Array,
    B_b2: jax.Array,
):
    return _impl(A_x, A_wqkv, A_wo, B_x, B_w1, B_b1, B_w2, B_b2)
```
